```python
import os as _os
_os.environ.setdefault("JAX_PLATFORMS", "cpu")
import jax
import jax.numpy as jnp

def _softmax(x, axis=-1):
    return jax.nn.softmax(x, axis=axis)
def _gelu(x):
    return jax.nn.gelu(x, approximate=True)
def _silu(x):
    return jax.nn.silu(x)
def _sigmoid(x):
    return jax.nn.sigmoid(x)
def _layernorm(x, axis=-1, eps=1e-5):
    m = jnp.mean(x, axis=axis, keepdims=True)
    v = jnp.var(x, axis=axis, keepdims=True)
    return (x - m) / jnp.sqrt(v + eps)
def _scatter_add(tgt, idx, src, axis=0):
    return tgt.at[idx].add(src)
def _segment_sum(src, seg, n):
    return jax.ops.segment_sum(src, seg, n)
class _Rng:
    def __init__(self, key):
        self._k = key
    def _next(self):
        self._k, sub = jax.random.split(self._k)
        return sub
    def normal(self, shape):
        return jax.random.normal(self._next(), shape, dtype=jnp.bfloat16)
    def randint(self, lo, hi, shape):
        return jax.random.randint(self._next(), shape, lo, hi, dtype=jnp.int32)
    def uniform(self, shape, lo=0.0, hi=1.0):
        return jax.random.uniform(self._next(), shape, jnp.bfloat16, lo, hi)
    def permutation(self, n):
        return jax.random.permutation(self._next(), n)


kernel_name = 'concat_heads__sliding_block_cached__sliding_block_cached__decode'

def setup_inputs():
    _rng = _Rng(jax.random.key(int.from_bytes(__import__("os").urandom(4), "little")))
    _w = (lambda a: (lambda t: t.astype(jnp.bfloat16) if jnp.issubdtype(t.dtype, jnp.floating) else t)(jnp.asarray(a)))
    def _A_setup():
        B, Sq, D = 2, 1, 640
        Hq, Hkv, Sk, Dh = 32, 32, 4096, 128
        assert Hq % Hkv == 0, (Hq, Hkv)
        return {
            "x": _w((lambda *s: _rng.normal(s) * 0.8)(B, Sq, D)),
            "k_cache": _w((lambda *s: _rng.normal(s) * 0.8)(B, Hkv, Sk, Dh)),
            "v_cache": _w((lambda *s: _rng.normal(s) * 0.05)(B, Hkv, Sk, Dh)),
            "wq": _w((lambda *s: _rng.normal(s) * 0.8)(D, Hq * Dh) * (D ** -0.5)),
            "wo": _w((lambda *s: _rng.normal(s) * 0.05)(Hq * Dh, D) * ((Hq * Dh) ** -0.5)),
        }
    _A_in = _A_setup()

    def _B_setup():
        B, Sq, D = 2, 1, 640
        Hq, Hkv, Sk, Dh = 32, 32, 4096, 128
        assert Hq % Hkv == 0, (Hq, Hkv)
        return {
            "x": _w((lambda *s: _rng.normal(s) * 0.8)(B, Sq, D)),
            "k_cache": _w((lambda *s: _rng.normal(s) * 0.8)(B, Hkv, Sk, Dh)),
            "v_cache": _w((lambda *s: _rng.normal(s) * 0.05)(B, Hkv, Sk, Dh)),
            "wq": _w((lambda *s: _rng.normal(s) * 0.8)(D, Hq * Dh) * (D ** -0.5)),
            "wo": _w((lambda *s: _rng.normal(s) * 0.05)(Hq * Dh, D) * ((Hq * Dh) ** -0.5)),
        }
    _B_in = _B_setup()

    return {
        "A_x": _A_in["x"],
        "A_k_cache": _A_in["k_cache"],
        "A_v_cache": _A_in["v_cache"],
        "A_wq": _A_in["wq"],
        "A_wo": _A_in["wo"],
        "B_x": _B_in["x"],
        "B_k_cache": _B_in["k_cache"],
        "B_v_cache": _B_in["v_cache"],
        "B_wq": _B_in["wq"],
        "B_wo": _B_in["wo"],
    }

def reference(A_x, A_k_cache, A_v_cache, A_wq, A_wo, B_x, B_k_cache, B_v_cache, B_wq, B_wo):
    def _A_ref(x, k_cache, v_cache, wq, wo):
        B, Sq, D = x.shape
        Hq, Dh = 32, 128
        Hkv, Sk = k_cache.shape[1], k_cache.shape[2]
        W = min(4096, max(256, Sk // 4))
        rep = Hq // Hkv
        q = (lambda x, *d: x.transpose(*d))((x @ wq).reshape(B, Sq, Hq, Dh), 0, 2, 1, 3)
        k = jnp.repeat(k_cache[:, :, Sk - W:, :], rep, axis=1)
        v = jnp.repeat(v_cache[:, :, Sk - W:, :], rep, axis=1)
        scores = jnp.einsum("bhqd,bhkd->bhqk", q, k) * (Dh ** -0.5)
        p = _softmax(scores, axis=-1)
        o = jnp.einsum("bhqk,bhkd->bhqd", p, v)
        return (lambda x, *d: x.transpose(*d))(o, 0, 2, 1, 3).reshape(B, Sq, Hq * Dh) @ wo

    def _B_ref(x, k_cache, v_cache, wq, wo):
        B, Sq, D = x.shape
        Hq, Dh = 32, 128
        Hkv, Sk = k_cache.shape[1], k_cache.shape[2]
        W = min(4096, max(256, Sk // 4))
        rep = Hq // Hkv
        q = (lambda x, *d: x.transpose(*d))((x @ wq).reshape(B, Sq, Hq, Dh), 0, 2, 1, 3)
        k = jnp.repeat(k_cache[:, :, Sk - W:, :], rep, axis=1)
        v = jnp.repeat(v_cache[:, :, Sk - W:, :], rep, axis=1)
        scores = jnp.einsum("bhqd,bhkd->bhqk", q, k) * (Dh ** -0.5)
        p = _softmax(scores, axis=-1)
        o = jnp.einsum("bhqk,bhkd->bhqd", p, v)
        return (lambda x, *d: x.transpose(*d))(o, 0, 2, 1, 3).reshape(B, Sq, Hq * Dh) @ wo

    a = _A_ref(A_x, A_k_cache, A_v_cache, A_wq, A_wo)
    b = _B_ref(B_x, B_k_cache, B_v_cache, B_wq, B_wo)
    return jnp.concatenate([a, b], axis=-1)
```

```python
import jax
import jax.numpy as jnp
from jax import lax
import jax.experimental.pallas as pl
import jax.experimental.pallas.tpu as pltpu

_NT = (((1,), (1,)), ((), ()))


@jax.jit
def pallas_concat_heads__sliding_block_cached__sliding_block_cached__decode_kernel(
    A_x: jax.Array,
    A_k_cache: jax.Array,
    A_v_cache: jax.Array,
    A_wq: jax.Array,
    A_wo: jax.Array,
    B_x: jax.Array,
    B_k_cache: jax.Array,
    B_v_cache: jax.Array,
    B_wq: jax.Array,
    B_wo: jax.Array,
):
    B, SQ, D = A_x.shape
    _, H, SK, DH = A_k_cache.shape
    assert SQ == 1 and B == 2 and A_wq.shape == (D, H * DH) and A_wo.shape == (H * DH, D)
    W = min(4096, max(256, SK // 4))
    G = 4
    R = B * G
    NS = H // G
    NSTEP = 2 * NS
    NSLOT = 2
    WOS = (G - 1, 1)
    WO_OFF = (0, G - 1)
    NC = 3 + len(WOS)
    scale = DH ** -0.5
    f32, bf16 = jnp.float32, jnp.bfloat16

    def kernel(xa, xb, ka, va, wqa, woa, kb, vb, wqb, wob, out_ref,
               k_buf, v_buf, wq_buf, wo_buf, x_in, x_scr, sem, x_sem):

        def copies(k_hbm, v_hbm, wq_hbm, wo_hbm, hg, slot):
            h0 = hg * G
            s0 = slot * NC
            cs = [
                pltpu.make_async_copy(wq_hbm.at[:, pl.ds(h0 * DH, G * DH)],
                                      wq_buf.at[slot], sem.at[s0]),
                pltpu.make_async_copy(k_hbm.at[:, pl.ds(h0, G), pl.ds(SK - W, W), :],
                                      k_buf.at[slot], sem.at[s0 + 1]),
                pltpu.make_async_copy(v_hbm.at[:, pl.ds(h0, G), pl.ds(SK - W, W), :],
                                      v_buf.at[slot], sem.at[s0 + 2]),
            ]
            for j, n in enumerate(WOS):
                cs.append(pltpu.make_async_copy(
                    wo_hbm.at[pl.ds((h0 + WO_OFF[j]) * DH, n * DH), :],
                    wo_buf.at[slot, pl.ds(WO_OFF[j] * DH, n * DH), :],
                    sem.at[s0 + 3 + j]))
            return cs

        def issue(s):
            slot = s % NSLOT

            @pl.when(s < NS)
            def _():
                for c in copies(ka, va, wqa, woa, s, slot):
                    c.start()

            @pl.when(jnp.logical_and(s >= NS, s < NSTEP))
            def _():
                for c in copies(kb, vb, wqb, wob, s - NS, slot):
                    c.start()

        xcs = [pltpu.make_async_copy(x, x_in.at[i], x_sem.at[i]) for i, x in enumerate((xa, xb))]
        for c in xcs:
            c.start()
        for c in copies(ka, va, wqa, woa, 0, 0):
            c.start()

        row_d = lax.broadcasted_iota(jnp.int32, (R, D), 0)
        row_h = lax.broadcasted_iota(jnp.int32, (R, DH), 0)
        row_w = lax.broadcasted_iota(jnp.int32, (R, W), 0)
        row_b = lax.broadcasted_iota(jnp.int32, (B, D), 0)

        for i in range(2):
            xcs[i].wait()
            xv = x_in[i].astype(f32)
            x0 = jnp.broadcast_to(xv[0:1], (R, D))
            x1 = jnp.broadcast_to(xv[1:2], (R, D))
            x_scr[i] = jnp.where(row_d < G, x0, x1).astype(bf16)

        def finalize(acc, blk):
            o0 = jnp.sum(jnp.where(row_d < G, acc, 0.0), axis=0, keepdims=True)
            o1 = jnp.sum(jnp.where(row_d >= G, acc, 0.0), axis=0, keepdims=True)
            res = jnp.where(row_b == 0, jnp.broadcast_to(o0, (B, D)), jnp.broadcast_to(o1, (B, D)))
            out_ref[:, pl.ds(blk * D, D)] = res.astype(out_ref.dtype)

        def step(s, acc):
            slot = s % NSLOT
            issue(s + 1)
            cs = copies(ka, va, wqa, woa, 0, slot)

            cs[0].wait()
            qall = jnp.dot(x_scr[s // NS], wq_buf[slot], preferred_element_type=f32)
            q8 = qall[:, 0:DH]
            for g in range(1, G):
                q8 = jnp.where(row_h % G == g, qall[:, g * DH:(g + 1) * DH], q8)
            q8 = q8.astype(bf16)

            cs[1].wait()
            sc = None
            for r in range(R):
                b, g = divmod(r, G)
                sr = lax.dot_general(q8, k_buf[slot, b, g], _NT, preferred_element_type=f32)
                sc = sr if sc is None else jnp.where(row_w == r, sr, sc)
            sc = sc * scale
            m = jnp.max(sc, axis=1, keepdims=True)
            p = jnp.exp(sc - m)
            inv_l = 1.0 / jnp.sum(p, axis=1, keepdims=True)
            pb = p.astype(bf16)

            cs[2].wait()
            o = None
            for r in range(R):
                b, g = divmod(r, G)
                orr = jnp.dot(pb, v_buf[slot, b, g], preferred_element_type=f32)
                o = orr if o is None else jnp.where(row_h == r, orr, o)
            ob = (o * inv_l).astype(bf16)

            acc = jnp.where(s == NS, 0.0, acc)
            for j, n in enumerate(WOS):
                cs[3 + j].wait()
                for g in range(WO_OFF[j], WO_OFF[j] + n):
                    rg = jnp.dot(ob, wo_buf[slot, pl.ds(g * DH, DH), :], preferred_element_type=f32)
                    acc = acc + jnp.where(row_d % G == g, rg, 0.0)

            @pl.when(s == NS - 1)
            def _():
                finalize(acc, 0)

            return acc

        acc = lax.fori_loop(0, NSTEP, step, jnp.zeros((R, D), f32))
        finalize(acc, 1)

    any_spec = pl.BlockSpec(memory_space=pl.ANY)
    out = pl.pallas_call(
        kernel,
        out_shape=jax.ShapeDtypeStruct((B, 2 * D), A_x.dtype),
        in_specs=[any_spec] * 10,
        out_specs=pl.BlockSpec(memory_space=pltpu.VMEM),
        scratch_shapes=[
            pltpu.VMEM((NSLOT, B, G, W, DH), bf16),
            pltpu.VMEM((NSLOT, B, G, W, DH), bf16),
            pltpu.VMEM((NSLOT, D, G * DH), bf16),
            pltpu.VMEM((NSLOT, G * DH, D), bf16),
            pltpu.VMEM((2, B, D), bf16),
            pltpu.VMEM((2, R, D), bf16),
            pltpu.SemaphoreType.DMA((NSLOT * NC,)),
            pltpu.SemaphoreType.DMA((2,)),
        ],
        compiler_params=pltpu.CompilerParams(vmem_limit_bytes=32 * 1024 * 1024),
    )(A_x.reshape(B, D), B_x.reshape(B, D),
      A_k_cache, A_v_cache, A_wq, A_wo, B_k_cache, B_v_cache, B_wq, B_wo)
    return out.reshape(B, SQ, 2 * D)
```

```python
import jax
import jax.numpy as jnp
from jax import lax
import jax.experimental.pallas as pl
import jax.experimental.pallas.tpu as pltpu

_NT = (((1,), (1,)), ((), ()))


@jax.jit
def pallas_concat_heads__sliding_block_cached__sliding_block_cached__decode_kernel(
    A_x: jax.Array,
    A_k_cache: jax.Array,
    A_v_cache: jax.Array,
    A_wq: jax.Array,
    A_wo: jax.Array,
    B_x: jax.Array,
    B_k_cache: jax.Array,
    B_v_cache: jax.Array,
    B_wq: jax.Array,
    B_wo: jax.Array,
):
    B, SQ, D = A_x.shape
    _, H, SK, DH = A_k_cache.shape
    assert SQ == 1 and B == 2 and A_wq.shape == (D, H * DH) and A_wo.shape == (H * DH, D)
    assert D % DH == 0
    W = min(4096, max(256, SK // 4))
    G = 4
    R = B * G
    NS = H // G
    NSTEP = 2 * NS
    NSLOT = 2
    LAST_SLOT = (NSTEP - 1) % NSLOT
    NP = 4
    PR = DH // NP
    NHEAD_ROWS = (G - 1) * DH
    scale = DH ** -0.5
    f32, bf16 = jnp.float32, jnp.bfloat16

    def kernel(xa, xb, ka, va, wqa, woa, kb, vb, wqb, wob, out_ref,
               k_buf, v_buf, wq_buf, wo_buf, x_in, x_scr, c_scr, sem, tail_sem, x_sem):

        def copies(k_hbm, v_hbm, wq_hbm, wo_hbm, hg, slot, last):
            h0 = hg * G
            s0 = slot * 4
            cs = [
                pltpu.make_async_copy(wq_hbm.at[:, pl.ds(h0 * DH, G * DH)],
                                      wq_buf.at[slot], sem.at[s0]),
                pltpu.make_async_copy(k_hbm.at[:, pl.ds(h0, G), pl.ds(SK - W, W), :],
                                      k_buf.at[slot], sem.at[s0 + 1]),
                pltpu.make_async_copy(v_hbm.at[:, pl.ds(h0, G), pl.ds(SK - W, W), :],
                                      v_buf.at[slot], sem.at[s0 + 2]),
            ]
            if not last:
                cs.append(pltpu.make_async_copy(wo_hbm.at[pl.ds(h0 * DH, G * DH), :],
                                                wo_buf.at[slot], sem.at[s0 + 3]))
            else:
                cs.append(pltpu.make_async_copy(wo_hbm.at[pl.ds(h0 * DH, NHEAD_ROWS), :],
                                                wo_buf.at[slot, pl.ds(0, NHEAD_ROWS), :],
                                                sem.at[s0 + 3]))
                for j in range(NP):
                    r0 = NHEAD_ROWS + j * PR
                    cs.append(pltpu.make_async_copy(wo_hbm.at[pl.ds(h0 * DH + r0, PR), :],
                                                    wo_buf.at[slot, pl.ds(r0, PR), :],
                                                    tail_sem.at[j]))
            return cs

        def issue(s):
            slot = s % NSLOT

            @pl.when(s < NS)
            def _():
                for c in copies(ka, va, wqa, woa, s, slot, False):
                    c.start()

            @pl.when(jnp.logical_and(s >= NS, s < NSTEP - 1))
            def _():
                for c in copies(kb, vb, wqb, wob, s - NS, slot, False):
                    c.start()

            @pl.when(s == NSTEP - 1)
            def _():
                for c in copies(kb, vb, wqb, wob, NS - 1, LAST_SLOT, True):
                    c.start()

        xcs = [pltpu.make_async_copy(x, x_in.at[i], x_sem.at[i]) for i, x in enumerate((xa, xb))]
        for c in xcs:
            c.start()
        for c in copies(ka, va, wqa, woa, 0, 0, False):
            c.start()

        row_d = lax.broadcasted_iota(jnp.int32, (R, D), 0)
        row_h = lax.broadcasted_iota(jnp.int32, (R, DH), 0)
        row_w = lax.broadcasted_iota(jnp.int32, (R, W), 0)
        row_b = lax.broadcasted_iota(jnp.int32, (B, D), 0)

        for i in range(2):
            xcs[i].wait()
            xv = x_in[i].astype(f32)
            x0 = jnp.broadcast_to(xv[0:1], (R, D))
            x1 = jnp.broadcast_to(xv[1:2], (R, D))
            x_scr[i] = jnp.where(row_d < G, x0, x1).astype(bf16)

        def two_rows(r0, r1):
            return jnp.where(row_b == 0, jnp.broadcast_to(r0, (B, D)), jnp.broadcast_to(r1, (B, D)))

        def reduce_rows(acc):
            return two_rows(jnp.sum(jnp.where(row_d < G, acc, 0.0), axis=0, keepdims=True),
                            jnp.sum(jnp.where(row_d >= G, acc, 0.0), axis=0, keepdims=True))

        def attend(cs, slot, blk):
            cs[0].wait()
            qall = jnp.dot(x_scr[blk], wq_buf[slot], preferred_element_type=f32)
            q8 = qall[:, 0:DH]
            for g in range(1, G):
                q8 = jnp.where(row_h % G == g, qall[:, g * DH:(g + 1) * DH], q8)
            q8 = q8.astype(bf16)

            cs[1].wait()
            sc = None
            for r in range(R):
                b, g = divmod(r, G)
                sr = lax.dot_general(q8, k_buf[slot, b, g], _NT, preferred_element_type=f32)
                sc = sr if sc is None else jnp.where(row_w == r, sr, sc)
            sc = sc * scale
            m = jnp.max(sc, axis=1, keepdims=True)
            p = jnp.exp(sc - m)
            inv_l = 1.0 / jnp.sum(p, axis=1, keepdims=True)
            pb = p.astype(bf16)

            cs[2].wait()
            o = None
            for r in range(R):
                b, g = divmod(r, G)
                orr = jnp.dot(pb, v_buf[slot, b, g], preferred_element_type=f32)
                o = orr if o is None else jnp.where(row_h == r, orr, o)
            return (o * inv_l).astype(bf16)

        def project(acc, ob, slot, heads):
            for g in heads:
                rg = jnp.dot(ob, wo_buf[slot, pl.ds(g * DH, DH), :], preferred_element_type=f32)
                acc = acc + jnp.where(row_d % G == g, rg, 0.0)
            return acc

        def step(s, acc):
            slot = s % NSLOT
            issue(s + 1)
            cs = copies(ka, va, wqa, woa, 0, slot, False)
            ob = attend(cs, slot, s // NS)
            acc = jnp.where(s == NS, 0.0, acc)
            cs[3].wait()
            acc = project(acc, ob, slot, range(G))

            @pl.when(s == NS - 1)
            def _():
                out_ref[:, pl.ds(0, D)] = reduce_rows(acc).astype(out_ref.dtype)

            return acc

        acc = lax.fori_loop(0, NSTEP - 1, step, jnp.zeros((R, D), f32))

        cs = copies(kb, vb, wqb, wob, NS - 1, LAST_SLOT, True)
        ob = attend(cs, LAST_SLOT, 1)
        of = ob.astype(f32)
        rr = lax.broadcasted_iota(jnp.int32, (DH, DH), 0)
        ll = lax.broadcasted_iota(jnp.int32, (DH, DH), 1)
        for b in range(B):
            r = b * G + G - 1
            dg = jnp.where(rr == ll, jnp.broadcast_to(of[r:r + 1], (DH, DH)), 0.0)
            c_scr[b] = jnp.broadcast_to(jnp.sum(dg, axis=1, keepdims=True), (DH, DH))
        cs[3].wait()
        part = reduce_rows(project(acc, ob, LAST_SLOT, range(G - 1)))
        t = [None] * B
        for j in range(NP):
            cs[4 + j].wait()
            w = wo_buf[LAST_SLOT, pl.ds(NHEAD_ROWS + j * PR, PR), :].astype(f32)
            for b in range(B):
                cb = c_scr[b, pl.ds(j * PR, PR), :]
                pr = w * jnp.tile(cb, (1, D // DH))
                pr = jnp.sum(pr.reshape(PR // 8, 8, D), axis=0)
                t[b] = pr if t[b] is None else t[b] + pr
        res = part + two_rows(jnp.sum(t[0], axis=0, keepdims=True),
                              jnp.sum(t[1], axis=0, keepdims=True))
        out_ref[:, pl.ds(D, D)] = res.astype(out_ref.dtype)

    params = dict(vmem_limit_bytes=32 * 1024 * 1024)
    if hasattr(pltpu.CompilerParams, "disable_semaphore_checks"):
        params["disable_semaphore_checks"] = True

    any_spec = pl.BlockSpec(memory_space=pl.ANY)
    out = pl.pallas_call(
        kernel,
        out_shape=jax.ShapeDtypeStruct((B, 2 * D), A_x.dtype),
        in_specs=[any_spec] * 10,
        out_specs=pl.BlockSpec(memory_space=pltpu.VMEM),
        scratch_shapes=[
            pltpu.VMEM((NSLOT, B, G, W, DH), bf16),
            pltpu.VMEM((NSLOT, B, G, W, DH), bf16),
            pltpu.VMEM((NSLOT, D, G * DH), bf16),
            pltpu.VMEM((NSLOT, G * DH, D), bf16),
            pltpu.VMEM((2, B, D), bf16),
            pltpu.VMEM((2, R, D), bf16),
            pltpu.VMEM((B, DH, DH), f32),
            pltpu.SemaphoreType.DMA((NSLOT * 4,)),
            pltpu.SemaphoreType.DMA((NP,)),
            pltpu.SemaphoreType.DMA((2,)),
        ],
        compiler_params=pltpu.CompilerParams(**params),
    )(A_x.reshape(B, D), B_x.reshape(B, D),
      A_k_cache, A_v_cache, A_wq, A_wo, B_k_cache, B_v_cache, B_wq, B_wo)
    return out.reshape(B, SQ, 2 * D)
```

```python
import numpy as np
import jax
import jax.numpy as jnp
from jax import lax
import jax.experimental.pallas as pl
import jax.experimental.pallas.tpu as pltpu

_NT = (((1,), (1,)), ((), ()))


@jax.jit
def pallas_concat_heads__sliding_block_cached__sliding_block_cached__decode_kernel(
    A_x: jax.Array,
    A_k_cache: jax.Array,
    A_v_cache: jax.Array,
    A_wq: jax.Array,
    A_wo: jax.Array,
    B_x: jax.Array,
    B_k_cache: jax.Array,
    B_v_cache: jax.Array,
    B_wq: jax.Array,
    B_wo: jax.Array,
):
    B, SQ, D = A_x.shape
    _, H, SK, DH = A_k_cache.shape
    assert SQ == 1 and B == 2 and A_wq.shape == (D, H * DH) and A_wo.shape == (H * DH, D)
    assert D % DH == 0
    W = min(4096, max(256, SK // 4))
    G = 4
    R = B * G
    NS = H // G
    assert H % G == 0 and NS >= 2
    NSTEP = 2 * NS
    NSLOT = 2
    LAST_SLOT = (NSTEP - 1) % NSLOT
    NP = 4
    PR = DH // NP
    NHEAD_ROWS = (G - 1) * DH
    scale = float(np.asarray(DH ** -0.5, dtype=jnp.bfloat16))
    f32, bf16 = jnp.float32, jnp.bfloat16

    def kernel(xa, xb, ka, va, wqa, woa, kb, vb, wqb, wob, out_ref,
               k_buf, v_buf, wq_buf, wo_buf, x_in, x_scr, c_scr, sem, tail_sem, x_sem):

        def copies(k_hbm, v_hbm, wq_hbm, wo_hbm, hg, slot, last):
            h0 = hg * G
            s0 = slot * 4
            cs = [
                pltpu.make_async_copy(wq_hbm.at[:, pl.ds(h0 * DH, G * DH)],
                                      wq_buf.at[slot], sem.at[s0]),
                pltpu.make_async_copy(k_hbm.at[:, pl.ds(h0, G), pl.ds(SK - W, W), :],
                                      k_buf.at[slot], sem.at[s0 + 1]),
                pltpu.make_async_copy(v_hbm.at[:, pl.ds(h0, G), pl.ds(SK - W, W), :],
                                      v_buf.at[slot], sem.at[s0 + 2]),
            ]
            if not last:
                cs.append(pltpu.make_async_copy(wo_hbm.at[pl.ds(h0 * DH, G * DH), :],
                                                wo_buf.at[slot], sem.at[s0 + 3]))
            else:
                cs.append(pltpu.make_async_copy(wo_hbm.at[pl.ds(h0 * DH, NHEAD_ROWS), :],
                                                wo_buf.at[slot, pl.ds(0, NHEAD_ROWS), :],
                                                sem.at[s0 + 3]))
                for j in range(NP):
                    r0 = NHEAD_ROWS + j * PR
                    cs.append(pltpu.make_async_copy(wo_hbm.at[pl.ds(h0 * DH + r0, PR), :],
                                                    wo_buf.at[slot, pl.ds(r0, PR), :],
                                                    tail_sem.at[j]))
            return cs

        def issue(s):
            slot = s % NSLOT

            @pl.when(s < NS)
            def _():
                for c in copies(ka, va, wqa, woa, s, slot, False):
                    c.start()

            @pl.when(jnp.logical_and(s >= NS, s < NSTEP - 1))
            def _():
                for c in copies(kb, vb, wqb, wob, s - NS, slot, False):
                    c.start()

            @pl.when(s == NSTEP - 1)
            def _():
                for c in copies(kb, vb, wqb, wob, NS - 1, LAST_SLOT, True):
                    c.start()

        xcs = [pltpu.make_async_copy(x, x_in.at[i], x_sem.at[i]) for i, x in enumerate((xa, xb))]
        for c in xcs:
            c.start()
        for c in copies(ka, va, wqa, woa, 0, 0, False):
            c.start()

        row_d = lax.broadcasted_iota(jnp.int32, (R, D), 0)
        row_h = lax.broadcasted_iota(jnp.int32, (R, DH), 0)
        row_w = lax.broadcasted_iota(jnp.int32, (R, W), 0)
        row_b = lax.broadcasted_iota(jnp.int32, (B, D), 0)

        for i in range(2):
            xcs[i].wait()
            xv = x_in[i].astype(f32)
            x0 = jnp.broadcast_to(xv[0:1], (R, D))
            x1 = jnp.broadcast_to(xv[1:2], (R, D))
            x_scr[i] = jnp.where(row_d < G, x0, x1).astype(bf16)

        def two_rows(r0, r1):
            return jnp.where(row_b == 0, jnp.broadcast_to(r0, (B, D)), jnp.broadcast_to(r1, (B, D)))

        def reduce_rows(acc):
            return two_rows(jnp.sum(jnp.where(row_d < G, acc, 0.0), axis=0, keepdims=True),
                            jnp.sum(jnp.where(row_d >= G, acc, 0.0), axis=0, keepdims=True))

        def attend(cs, slot, blk):
            cs[0].wait()
            qall = jnp.dot(x_scr[blk], wq_buf[slot], preferred_element_type=f32)
            q8 = qall[:, 0:DH]
            for g in range(1, G):
                q8 = jnp.where(row_h % G == g, qall[:, g * DH:(g + 1) * DH], q8)
            q8 = q8.astype(bf16)

            cs[1].wait()
            sc = None
            for r in range(R):
                b, g = divmod(r, G)
                sr = lax.dot_general(q8, k_buf[slot, b, g], _NT, preferred_element_type=f32)
                sc = sr if sc is None else jnp.where(row_w == r, sr, sc)
            sc = (sc.astype(bf16).astype(f32) * scale).astype(bf16).astype(f32)
            m = jnp.max(sc, axis=1, keepdims=True)
            p = jnp.exp(sc - m)
            inv_l = 1.0 / jnp.sum(p, axis=1, keepdims=True)
            pb = p.astype(bf16)

            cs[2].wait()
            o = None
            for r in range(R):
                b, g = divmod(r, G)
                orr = jnp.dot(pb, v_buf[slot, b, g], preferred_element_type=f32)
                o = orr if o is None else jnp.where(row_h == r, orr, o)
            return (o * inv_l).astype(bf16)

        def project(acc, ob, slot, heads):
            for g in heads:
                rg = jnp.dot(ob, wo_buf[slot, pl.ds(g * DH, DH), :], preferred_element_type=f32)
                acc = acc + jnp.where(row_d % G == g, rg, 0.0)
            return acc

        def step(s, acc):
            slot = s % NSLOT
            issue(s + 1)
            cs = copies(ka, va, wqa, woa, 0, slot, False)
            ob = attend(cs, slot, s // NS)
            acc = jnp.where(s == NS, 0.0, acc)
            cs[3].wait()
            acc = project(acc, ob, slot, range(G))

            @pl.when(s == NS - 1)
            def _():
                out_ref[:, pl.ds(0, D)] = reduce_rows(acc).astype(out_ref.dtype)

            return acc

        acc = lax.fori_loop(0, NSTEP - 1, step, jnp.zeros((R, D), f32))

        cs = copies(kb, vb, wqb, wob, NS - 1, LAST_SLOT, True)
        ob = attend(cs, LAST_SLOT, 1)
        of = ob.astype(f32)
        rr = lax.broadcasted_iota(jnp.int32, (DH, DH), 0)
        ll = lax.broadcasted_iota(jnp.int32, (DH, DH), 1)
        for b in range(B):
            r = b * G + G - 1
            dg = jnp.where(rr == ll, jnp.broadcast_to(of[r:r + 1], (DH, DH)), 0.0)
            c_scr[b] = jnp.broadcast_to(jnp.sum(dg, axis=1, keepdims=True), (DH, DH))
        cs[3].wait()
        part = reduce_rows(project(acc, ob, LAST_SLOT, range(G - 1)))
        t = [None] * B
        for j in range(NP):
            cs[4 + j].wait()
            w = wo_buf[LAST_SLOT, pl.ds(NHEAD_ROWS + j * PR, PR), :].astype(f32)
            for b in range(B):
                cb = c_scr[b, pl.ds(j * PR, PR), :]
                pr = w * jnp.tile(cb, (1, D // DH))
                pr = jnp.sum(pr.reshape(PR // 8, 8, D), axis=0)
                t[b] = pr if t[b] is None else t[b] + pr
        res = part + two_rows(jnp.sum(t[0], axis=0, keepdims=True),
                              jnp.sum(t[1], axis=0, keepdims=True))
        out_ref[:, pl.ds(D, D)] = res.astype(out_ref.dtype)

    params = dict(vmem_limit_bytes=32 * 1024 * 1024)
    if hasattr(pltpu.CompilerParams, "disable_semaphore_checks"):
        params["disable_semaphore_checks"] = True

    any_spec = pl.BlockSpec(memory_space=pl.ANY)
    out = pl.pallas_call(
        kernel,
        out_shape=jax.ShapeDtypeStruct((B, 2 * D), A_x.dtype),
        in_specs=[any_spec] * 10,
        out_specs=pl.BlockSpec(memory_space=pltpu.VMEM),
        scratch_shapes=[
            pltpu.VMEM((NSLOT, B, G, W, DH), bf16),
            pltpu.VMEM((NSLOT, B, G, W, DH), bf16),
            pltpu.VMEM((NSLOT, D, G * DH), bf16),
            pltpu.VMEM((NSLOT, G * DH, D), bf16),
            pltpu.VMEM((2, B, D), bf16),
            pltpu.VMEM((2, R, D), bf16),
            pltpu.VMEM((B, DH, DH), f32),
            pltpu.SemaphoreType.DMA((NSLOT * 4,)),
            pltpu.SemaphoreType.DMA((NP,)),
            pltpu.SemaphoreType.DMA((2,)),
        ],
        compiler_params=pltpu.CompilerParams(**params),
    )(A_x.reshape(B, D), B_x.reshape(B, D),
      A_k_cache, A_v_cache, A_wq, A_wo, B_k_cache, B_v_cache, B_wq, B_wo)
    return out.reshape(B, SQ, 2 * D)
```
